```python
import os as _os
_os.environ.setdefault("JAX_PLATFORMS", "cpu")
import jax
import jax.numpy as jnp

def _softmax(x, axis=-1):
    return jax.nn.softmax(x, axis=axis)
def _gelu(x):
    return jax.nn.gelu(x, approximate=True)
def _silu(x):
    return jax.nn.silu(x)
def _sigmoid(x):
    return jax.nn.sigmoid(x)
def _layernorm(x, axis=-1, eps=1e-5):
    m = jnp.mean(x, axis=axis, keepdims=True)
    v = jnp.var(x, axis=axis, keepdims=True)
    return (x - m) / jnp.sqrt(v + eps)
def _scatter_add(tgt, idx, src, axis=0):
    return tgt.at[idx].add(src)
def _segment_sum(src, seg, n):
    return jax.ops.segment_sum(src, seg, n)
class _Rng:
    def __init__(self, key):
        self._k = key
    def _next(self):
        self._k, sub = jax.random.split(self._k)
        return sub
    def normal(self, shape):
        return jax.random.normal(self._next(), shape, dtype=jnp.bfloat16)
    def randint(self, lo, hi, shape):
        return jax.random.randint(self._next(), shape, lo, hi, dtype=jnp.int32)
    def uniform(self, shape, lo=0.0, hi=1.0):
        return jax.random.uniform(self._next(), shape, jnp.bfloat16, lo, hi)
    def permutation(self, n):
        return jax.random.permutation(self._next(), n)


kernel_name = 'interleave_layers__sliding_local_dilated__linear_kernel_hedgehog__prompt'

def setup_inputs():
    _rng = _Rng(jax.random.key(int.from_bytes(__import__("os").urandom(4), "little")))
    _w = (lambda a: (lambda t: t.astype(jnp.bfloat16) if jnp.issubdtype(t.dtype, jnp.floating) else t)(jnp.asarray(a)))
    def _A_setup():
        B, S, D = 1, 2048, 640
        return {
            "x": _w((lambda *s: _rng.normal(s) * 0.05)(B, S, D)),
            "wqkv": _w((lambda *s: _rng.normal(s) * 0.05)(D, 3 * D)),
            "wo": _w((lambda *s: _rng.normal(s) * 0.05)(D, D)),
        }
    _A_in = _A_setup()

    def _B_setup():
        B, S, D, H = 1, 2048, 640, 32
        Dh = D // H
        return {
            "x": _w((lambda *s: _rng.normal(s) * 0.05)(B, S, D)),
            "wqkv": _w((lambda *s: _rng.normal(s) * 0.4)(D, 3 * D)),
            "w_phi": _w((lambda *s: _rng.normal(s) * 0.4)(H, Dh, Dh) * (Dh ** -0.5)),
            "wo": _w((lambda *s: _rng.normal(s) * 0.1)(D, D)),
        }
    _B_in = _B_setup()

    return {
        "A_x": _A_in["x"],
        "A_wqkv": _A_in["wqkv"],
        "A_wo": _A_in["wo"],
        "B_x": _B_in["x"],
        "B_wqkv": _B_in["wqkv"],
        "B_w_phi": _B_in["w_phi"],
        "B_wo": _B_in["wo"],
    }

def reference(A_x, A_wqkv, A_wo, B_x, B_wqkv, B_w_phi, B_wo):
    def _A_ref(x, wqkv, wo):
        B, S, D = x.shape
        H = 32; Dh = D // H
        W, dil = 8, 2
        qkv = (lambda x, *d: x.transpose(*d))((x @ wqkv).reshape(B, S, 3, H, Dh), 2, 0, 3, 1, 4)
        q, k, v = qkv[0], qkv[1], qkv[2]
        scale = Dh ** -0.5
        pos = jnp.arange(S)
        off = jnp.arange(W) * dil
        idx = pos[:, None] - off[None, :]
        mask = idx >= 0
        idx_c = jnp.where(mask, idx, 0).reshape(-1)
        kg = k[:, :, idx_c, :].reshape(B, H, S, W, Dh)
        vg = v[:, :, idx_c, :].reshape(B, H, S, W, Dh)
        logits = jnp.einsum("bhsd,bhswd->bhsw", q, kg) * scale
        logits = jnp.where(mask[None, None, :, :], logits, -1e9)
        attn = _softmax(logits, axis=-1)
        o = jnp.einsum("bhsw,bhswd->bhsd", attn, vg)
        return (lambda x, *d: x.transpose(*d))(o, 0, 2, 1, 3).reshape(B, S, D) @ wo

    def _B_ref(x, wqkv, w_phi, wo):
        B, S, D = x.shape
        H = 32; Dh = D // H
        qkv = (lambda x, *d: x.transpose(*d))((x @ wqkv).reshape(B, S, 3, H, Dh), 2, 0, 3, 1, 4)
        q, k, v = qkv[0], qkv[1], qkv[2]
        pq = jnp.einsum("bhsd,hdf->bhsf", q, w_phi)
        pk = jnp.einsum("bhsd,hdf->bhsf", k, w_phi)
        phi_q = jnp.concatenate([_softmax(pq, axis=-1), _softmax(-pq, axis=-1)], axis=-1)
        phi_k = jnp.concatenate([_softmax(pk, axis=-1), _softmax(-pk, axis=-1)], axis=-1)
        kv = jnp.einsum("bhsf,bhsd->bhfd", phi_k, v)
        z  = jnp.einsum("bhsf->bhf", phi_k)
        num = jnp.einsum("bhqf,bhfd->bhqd", phi_q, kv)
        den = jnp.einsum("bhqf,bhf->bhq", phi_q, z)[..., None] + 1e-6
        o = num / den
        return (lambda x, *d: x.transpose(*d))(o, 0, 2, 1, 3).reshape(B, S, D) @ wo

    x = A_x
    x = x + _A_ref(_layernorm(x, axis=-1), A_wqkv, A_wo)
    x = x + _B_ref(_layernorm(x, axis=-1), B_wqkv, B_w_phi, B_wo)
    x = x + _A_ref(_layernorm(x, axis=-1), A_wqkv, A_wo)
    x = x + _B_ref(_layernorm(x, axis=-1), B_wqkv, B_w_phi, B_wo)
    return x
```

```python
import functools
import jax
import jax.numpy as jnp
import numpy as np
from jax import lax
import jax.experimental.pallas as pl
import jax.experimental.pallas.tpu as pltpu

S, D, H, DH = 2048, 640, 32, 20
W, NT, T = 8, 16, 128
HALO = W - 1
CHUNK = 640
DP = D // 2
LOG2E = 1.4426950408889634
F32, BF16 = jnp.float32, jnp.bfloat16
INTERPRET = False


def _iota(shape, d):
    return lax.broadcasted_iota(jnp.int32, shape, d)


def _rcp(x):
    r = pl.reciprocal(x, approx=True)
    return r * (2.0 - x * r)


def _dot(a, b):
    return jnp.dot(a, b, preferred_element_type=F32)


def _dot_nt(a, b):
    return lax.dot_general(a, b, (((1,), (1,)), ((), ())), preferred_element_type=F32)


def _tree(op, xs):
    xs = list(xs)
    while len(xs) > 1:
        xs = [op(xs[i], xs[i + 1]) if i + 1 < len(xs) else xs[i] for i in range(0, len(xs), 2)]
    return xs[0]


def _pipeline(stages, lo, hi):
    n = len(stages)

    def step(i, par, active):
        live = []
        for k, st in enumerate(stages):
            if active(k):
                g = st(i - k, (par - k) % 2)
                live.append([0.0, next(g), g, ORDER(k)])
        while live:
            e = min(live, key=lambda v: ((v[0] + v[3]) / v[1]))
            e[0] += 1
            next(e[2], None)
            if e[0] == e[1]:
                for _ in e[2]:
                    pass
                live.remove(e)

    first = lo + n - 1
    for i in range(lo, min(first, hi + n - 1)):
        step(i, i % 2, lambda k: lo <= i - k < hi)
    pairs = max(hi - first, 0) // 2
    if pairs:
        def body(t, c):
            i = first + 2 * t
            step(i, first % 2, lambda k: True)
            step(i + 1, (first + 1) % 2, lambda k: True)
            return c
        if pairs == 1:
            body(0, 0)
        else:
            lax.fori_loop(0, pairs, body, 0)
    for i in range(first + 2 * pairs, hi + n - 1):
        step(i, i % 2, lambda k: lo <= i - k < hi)


def ORDER(k):
    return 0.5


def _both(f):
    def st(j, s):
        g = [f(2 * j + u, s, u) for u in range(2)]
        n = next(g[0]) + next(g[1])
        yield n
        for it in g:
            for _ in it:
                yield
            yield
    return st


def _kernel(x_hbm, wa_hbm, woa_hbm, wb_hbm, wphi_ref, wob_hbm, out_hbm,
            xio, wa, woa, wb, wob, wat, woat, wbt, wobt, wtmp, pt0, pt1, wp32,
            X, XN, Kb, Vb, Q0, Q1, O0, O1, T0, T1, P0, P1, F0, F1, V0, V1, V2, V3,
            acc, zacc, kvt, zf, sems):
    Qs, Os, Ts, Ps, Fs, Vs = (Q0, Q1), (O0, O1), (T0, T1), (P0, P1), (F0, F1), (V0, V1, V2, V3)

    cp_x = [pltpu.make_async_copy(x_hbm.at[:, pl.ds(i * T, T)], xio.bitcast(BF16).at[pl.ds(i * S, S)], sems.at[0]) for i in range(5)]

    def wcopy(hbm, buf, tiles, sem):
        return [pltpu.make_async_copy(hbm.at[:, pl.ds(i * T, T)], buf.at[pl.ds(i * D, D)], sems.at[sem])
                for i in tiles]

    cp_wkv, cp_wq = wcopy(wa_hbm, wa, range(5, 15), 1), wcopy(wa_hbm, wa, range(5), 5)
    cp_rest = (wcopy(woa_hbm, woa, range(5), 2) + wcopy(wb_hbm, wb, range(15), 3)
               + wcopy(wob_hbm, wob, range(5), 4))
    for c_ in cp_wkv + cp_wq + cp_x:
        c_.start()

    def wmat(ref, nblk, b0, b1):
        m = ref.shape[0] // 5
        return jnp.concatenate([pltpu.bitcast(ref[t * m + b0 * DP:t * m + b1 * DP, :], BF16) for t in range(5)], axis=1)

    def put(dst, row, y):
        dst[row // 2:(row + y.shape[0]) // 2, :] = pltpu.bitcast(y.astype(BF16), jnp.int32)

    def bands(n):
        out, m = [], n * DH
        for t in range(5):
            q0, q1 = (t * T) // m, (t * T + T - 1) // m
            shp = ((q1 - q0 + 1) * m, T)
            r, c = _iota(shp, 0), _iota(shp, 1)
            qq = (r >= m).astype(jnp.int32) + (r >= 2 * m)
            src = (n * (q0 + qq) + (r & (n - 1))) * DH + ((r - m * qq) >> (n.bit_length() - 1))
            out.append((q0, q1, jnp.where(c + t * T == src, 1.0, 0.0).astype(BF16)))
        return out

    def apply(band, mm):
        m = D // (band[-1][1] + 1)
        parts = [[] for _ in range(D // m)]
        for t, (q0, q1, bd) in enumerate(band):
            y = mm(bd, t)
            for q in range(q0, q1 + 1):
                parts[q].append(y[(q - q0) * m:(q - q0 + 1) * m])
        return jnp.concatenate([_tree(jnp.add, p) for p in parts], axis=0).astype(BF16)

    def prep_in(src, blk, band, dst):
        y = apply(band, lambda bd, t: _dot_nt(bd, src[(5 * blk + t) * D:(5 * blk + t + 1) * D, :]))
        for t in range(5):
            put(dst, t * 3 * D + blk * D, y[:, t * T:(t + 1) * T])

    def prep_out(src, band, dst):
        y = apply(band, lambda bd, t: _dot(bd, jnp.concatenate(
            [src[n * D + t * T:n * D + (t + 1) * T, :] for n in range(5)], axis=1)))
        for t in range(5):
            put(dst, t * D, y[t * T:(t + 1) * T, :].T)

    octet = bands(8)

    def prep_rest():
        for c_ in cp_rest:
            c_.wait()
        for h in range(H):
            wp32[h * DH:(h + 1) * DH, 0:DH] = wphi_ref[h].astype(F32)
        band = []
        for t in range(5):
            q0, q1 = (t * T) // 80, (t * T + T - 1) // 80
            n = (q1 - q0 + 1) * 80
            r, c = _iota((n, T), 0), _iota((n, T), 1)
            qq = (r >= 80).astype(jnp.int32) + (r >= 160)
            sel = (c == ((r - 80 * qq) >> 2)).astype(BF16)
            wp = jnp.where(_iota((T, T), 1) < DH, wp32[t * T:(t + 1) * T, :], 0.0).astype(BF16)
            lo = (4 * (q0 + qq) + (r & 3)) * DH - t * T
            bd = jnp.where((c >= lo) & (c < lo + DH), _dot_nt(sel, wp), 0.0).astype(BF16)
            band.append((q0, q1, bd))
        band = [(a, b, (c.astype(F32) * LOG2E).astype(BF16)) for a, b, c in band]
        prep_in(wb, 0, band, wbt)
        prep_in(wb, 1, band, wbt)
        quad = bands(4)
        prep_in(wb, 2, quad, wbt)
        prep_out(woa, octet, woat)
        prep_out(wob, quad, wobt)

    for c_ in cp_wkv:
        c_.wait()
    prep_in(wa, 1, octet, wat)
    prep_in(wa, 2, octet, wat)
    for c_ in cp_wq:
        c_.wait()
    prep_in(wa, 0, octet, wat)

    L = lambda u: slice(u * T, (u + 1) * T)
    CH = CHUNK
    two = lambda R, j, rs: jnp.concatenate([R[2 * j, rs, :], R[2 * j + 1, rs, :]], axis=1)

    def proj(ref, nblk, r0, nrows, rhs, sink):
        m = ref.shape[0] // 5
        yield nrows // CH
        for r in range(0, nrows, CH):
            w = jnp.concatenate([pltpu.bitcast(ref[t * m + (r0 + r) // 2:t * m + (r0 + r + CH) // 2, :], BF16)
                                 for t in range(5)], axis=1)
            sink(r, _dot(w, rhs()))
            yield

    @_both
    def ln(j, s, u):
        yield 2
        rows = [Ts[s][8 * i:8 * i + 8, L(u)] for i in range(D // 8)]
        add4 = lambda v: _tree(jnp.add, [functools.reduce(jnp.add, v[i::4]) for i in range(4)])
        m = jnp.sum(add4(rows), axis=0, keepdims=True) * (1.0 / D)
        var = jnp.sum(add4([(v - m) * (v - m) for v in rows]), axis=0, keepdims=True) * (1.0 / D)
        inv = lax.rsqrt(var + 1e-5)
        m = jnp.broadcast_to(m, (16, T))
        yield
        for i in range(D // 16):
            x = Ts[s][16 * i:16 * i + 16, L(u)]
            X[j, 16 * i:16 * i + 16, :] = x
            XN[j, 16 * i:16 * i + 16, :] = ((x - m) * inv).astype(BF16)
        yield

    @_both
    def load_x(j, s, u):
        yield 5
        for i in range(5):
            v = xio[pl.ds(i * (S // 2) + j, T // 2, stride=NT), :]
            Ts[s][i * T:(i + 1) * T, L(u)] = pltpu.bitcast(v, BF16).T.astype(F32)
            yield

    @_both
    def store_out(j, s, u):
        yield 5
        for i in range(5):
            y = Ts[s][i * T:(i + 1) * T, L(u)].astype(BF16).T
            xio[pl.ds(i * (S // 2) + j, T // 2, stride=NT), :] = pltpu.bitcast(y, jnp.int32)
            yield

    def out_proj(wt_ref):
        def st(j, s):
            def sink(r, y):
                Ts[s][r:r + CH, :] = two(X, j, slice(r, r + CH)) + y
            return proj(wt_ref, 1, 0, D, lambda: Os[s][...], sink)
        return st

    def a_kv(halo):
        def st(j, s):
            def sink(r, y):
                dst, r = (Kb, r) if r < D else (Vb, r - D)
                for u in range(2):
                    dst[2 * j + u + W, r:r + CH, :] = y[:, L(u)]
                    if halo:
                        dst[2 * j + u - W, r:r + CH, :] = pltpu.roll(y[:, L(u)], 2, 1)
            return proj(wat, 3, D, 2 * D, lambda: two(XN, j, slice(None)), sink)
        return st

    def to_p(ref):
        def st(j, s):
            def sink(r, y):
                Ps[s][r:r + CH, :] = y
            return proj(ref, 3, 0, D, lambda: two(XN, j, slice(None)), sink)
        return st

    def a_att(j, s):
        yield 20
        lane = _iota((8, T), 1)

        def logits(g):
            lg = [[None] * W for _ in range(2)]
            for d in range(DH):
                rs = slice(g * 160 + 8 * d, g * 160 + 8 * d + 8)
                k = [Kb[2 * j + 1 + i, rs, :] for i in range(W + 1)]
                for u in range(2):
                    q = Ps[s][rs, L(u)]
                    for w in range(W):
                        p = q * k[u + W - 1 - w]
                        lg[u][w] = p if d == 0 else lg[u][w] + p
                if d % 5 == 4:
                    yield
            res.append([soft(lg[u], 2 * j + u) for u in range(2)])

        def soft(lg, t):
            lg = [l * (DH ** -0.5 * LOG2E) for l in lg]
            lg = [jnp.where(lane < jnp.where(w > t, 2, 0), -1e9 * LOG2E, l) if w else l for w, l in enumerate(lg)]
            m = _tree(jnp.maximum, lg)
            e = [jnp.exp2(l - m) for l in lg]
            inv = _rcp(_tree(jnp.add, e))
            return [v * inv for v in e]

        def mix(g):
            for d in range(0, DH, 2):
                o = [[], []]
                for dd in (d, d + 1):
                    rs = slice(g * 160 + 8 * dd, g * 160 + 8 * dd + 8)
                    v = [Vb[2 * j + 1 + i, rs, :] for i in range(W + 1)]
                    for u in range(2):
                        o[u].append(functools.reduce(jnp.add, [res[g][u][w] * v[u + W - 1 - w] for w in range(W)]))
                for u in range(2):
                    Os[s][g * 160 + 8 * d:g * 160 + 8 * d + 16, L(u)] = jnp.concatenate(o[u], axis=0).astype(BF16)

        res = []
        for g in range(4):
            yield from logits(g)
            mix(g)
            yield

    def dual_softmax(p):
        rows = [p[8 * i:8 * i + 8] for i in range(10)]
        mx, mn = _tree(jnp.maximum, rows), _tree(jnp.minimum, rows)
        mx = jnp.maximum(mx, pltpu.roll(mx, 4, 0))
        mn = jnp.minimum(mn, pltpu.roll(mn, 4, 0))
        ep, en = [jnp.exp2(v - mx) for v in rows], [jnp.exp2(mn - v) for v in rows]
        sp, sn = _tree(jnp.add, ep), _tree(jnp.add, en)
        return ep, en, sp + pltpu.roll(sp, 4, 0), sn + pltpu.roll(sn, 4, 0)

    def b_kv_proj(j, s):
        def sink(r, y):
            if r < D:
                Ps[s][r:r + CH, :] = y
            else:
                Vs[s + 2 * cnt(s)][r - D:r - D + CH, :] = y.astype(BF16)
        return proj(wbt, 3, D, 2 * D, lambda: two(XN, j, slice(None)), sink)

    def cnt(s):
        return 0

    def b_k_soft(j, s):
        yield 8
        Vs[s + 2][...] = Vs[s][...]
        for q in range(8):
            phis = []
            for u in range(2):
                ep, en, sp, sn = dual_softmax(Ps[s][q * 80:(q + 1) * 80, L(u)])
                ip, im = _rcp(sp), _rcp(sn)
                phi = jnp.concatenate([v * ip for v in ep] + [v * im for v in en], axis=0)
                phis.append(phi)
                Fs[s][q * 160:(q + 1) * 160, L(u)] = phi.astype(BF16)
            zacc[q * 160:(q + 1) * 160, :] += phis[0] + phis[1]
            yield

    tiles_of = [list(range((160 * q) // T, (160 * q + 159) // T + 1)) for q in range(8)]

    def b_kv(j, s):
        yield 8
        for q in range(8):
            t0 = tiles_of[q][0]
            acc[q] += _dot_nt(Vs[s + 2][q * 80:(q + 1) * 80, :], Fs[s][t0 * T:(t0 + 2) * T, :])
            yield

    def b_fin():
        rr, lane = _iota((80, 2 * T), 0), _iota((80, 2 * T), 1)
        for q in range(8):
            off = 160 * q - tiles_of[q][0] * T
            ok = ((rr & 3) == (lane & 3)) & (lane >= off) & (lane < off + 160)
            kvt[q] = jnp.where(ok, acc[q], 0.0).astype(BF16)
        zf[...] = jnp.broadcast_to(jnp.sum(zacc[...], axis=1, keepdims=True), (2 * D, T))

    @_both
    def b_q_soft(j, s, u):
        yield 8
        for q in range(8):
            ep, en, sp, sn = dual_softmax(Ps[s][q * 80:(q + 1) * 80, L(u)])
            z = [zf[q * 160 + 8 * i:q * 160 + 8 * i + 8, :] for i in range(20)]
            dp = _tree(jnp.add, [a * b for a, b in zip(ep, z[:10])])
            dn = _tree(jnp.add, [a * b for a, b in zip(en, z[10:])])
            dp, dn = dp + pltpu.roll(dp, 4, 0), dn + pltpu.roll(dn, 4, 0)
            rp, rn = _rcp(sp), _rcp(sn)
            rd = _rcp(dp * rp + dn * rn + 1e-6)
            ip, im = rp * rd, rn * rd
            phi = jnp.concatenate([v * ip for v in ep] + [v * im for v in en], axis=0)
            Fs[s][q * 160:(q + 1) * 160, L(u)] = phi.astype(BF16)
            yield

    def b_num(j, s):
        yield 8
        for q in range(8):
            t0 = tiles_of[q][0]
            Os[s][q * 80:(q + 1) * 80, :] = _dot(kvt[q], Fs[s][t0 * T:(t0 + 2) * T, :]).astype(BF16)
            yield

    for c_ in cp_x:
        c_.wait()
    for c_ in cp_rest:
        c_.start()
    _pipeline([load_x, ln, a_kv(True)], W // 2, NT // 2)
    _pipeline([load_x, ln, a_kv(False)], 0, W // 2)
    prep_rest()

    def pair(it, carry):
        _pipeline([to_p(wat), a_att, out_proj(woat), ln], 0, NT // 2)
        acc[...] = jnp.zeros(acc.shape, F32)
        zacc[...] = jnp.zeros(zacc.shape, F32)
        _pipeline([b_kv_proj, b_k_soft, b_kv], 0, NT // 2)
        b_fin()

        @pl.when(it == 0)
        def _():
            _pipeline([to_p(wbt), b_q_soft, b_num, out_proj(wobt), ln], 0, NT // 2)
            _pipeline([a_kv(True)], W // 2, NT // 2)
            _pipeline([a_kv(False)], 0, W // 2)

        @pl.when(it == 1)
        def _():
            _pipeline([to_p(wbt), b_q_soft, b_num, out_proj(wobt), store_out], 0, NT // 2)
        return carry

    lax.fori_loop(0, 2, pair, 0)
    cp_o = [pltpu.make_async_copy(xio.bitcast(BF16).at[pl.ds(i * S, S)], out_hbm.at[:, pl.ds(i * T, T)], sems.at[0]) for i in range(5)]
    for c_ in cp_o:
        c_.start()
    for c_ in cp_o:
        c_.wait()


@jax.jit
def pallas_interleave_layers__sliding_local_dilated__linear_kernel_hedgehog__prompt_kernel(
    A_x: jax.Array,
    A_wqkv: jax.Array,
    A_wo: jax.Array,
    B_x: jax.Array,
    B_wqkv: jax.Array,
    B_w_phi: jax.Array,
    B_wo: jax.Array,
):
    del B_x
    hbm = pl.BlockSpec(memory_space=pl.ANY)
    vm = pltpu.VMEM
    tile = lambda rows, dt: [vm((rows, 2 * T), dt)] * 2
    out = pl.pallas_call(
        _kernel,
        out_shape=jax.ShapeDtypeStruct((S, D), BF16),
        in_specs=[hbm, hbm, hbm, hbm, pl.BlockSpec(memory_space=pltpu.VMEM), hbm],
        out_specs=hbm,
        scratch_shapes=[
            vm((5 * S // 2, T), jnp.int32), vm((15 * D, T), BF16), vm((5 * D, T), BF16), vm((15 * D, T), BF16), vm((5 * D, T), BF16),
            *([vm((15 * DP, T), jnp.int32), vm((5 * DP, T), jnp.int32)] * 2), vm((5 * DP, T), jnp.int32), *([vm((D, T), F32)] * 3),
            vm((NT, D, T), F32), vm((NT, D, T), BF16),
            vm((NT + W, D, T), F32), vm((NT + W, D, T), F32),
            *tile(D, F32), *tile(D, BF16), *tile(D, F32), *tile(D, F32), *tile(2 * D, BF16), *tile(D, BF16), *tile(D, BF16),
            vm((8, 80, 2 * T), F32), vm((2 * D, T), F32), vm((8, 80, 2 * T), BF16), vm((2 * D, T), F32),
            pltpu.SemaphoreType.DMA((6,)),
        ],
        compiler_params=pltpu.CompilerParams(vmem_limit_bytes=110 << 20),
        interpret=INTERPRET,
    )(A_x.reshape(S, D), A_wqkv, A_wo, B_wqkv, B_w_phi, B_wo)
    return out.reshape(A_x.shape)
```
